```python
import jax
import jax.numpy as jnp

def _softmax(x, axis=-1):
    return jax.nn.softmax(x, axis=axis)
def _gelu(x):
    return jax.nn.gelu(x, approximate=True)
def _silu(x):
    return jax.nn.silu(x)
def _sigmoid(x):
    return jax.nn.sigmoid(x)
def _layernorm(x, axis=-1, eps=1e-5):
    m = jnp.mean(x, axis=axis, keepdims=True)
    v = jnp.var(x, axis=axis, keepdims=True)
    return (x - m) / jnp.sqrt(v + eps)
def _scatter_add(tgt, idx, src, axis=0):
    return tgt.at[idx].add(src)
def _segment_sum(src, seg, n):
    return jax.ops.segment_sum(src, seg, n)
class _Rng:
    def __init__(self, key):
        self._k = key
    def _next(self):
        self._k, sub = jax.random.split(self._k)
        return sub
    def normal(self, shape):
        return jax.random.normal(self._next(), shape, dtype=jnp.bfloat16)
    def randint(self, lo, hi, shape):
        return jax.random.randint(self._next(), shape, lo, hi, dtype=jnp.int32)
    def uniform(self, shape, lo=0.0, hi=1.0):
        return jax.random.uniform(self._next(), shape, jnp.bfloat16, lo, hi)
    def permutation(self, n):
        return jax.random.permutation(self._next(), n)


kernel_name = 'recurrent_scan__sliding_block_cached__glu_gated_glu__decode'

def setup_inputs():
    _rng = _Rng(jax.random.key(int.from_bytes(__import__("os").urandom(4), "little")))
    _w = (lambda a: (lambda t: t.astype(jnp.bfloat16) if jnp.issubdtype(t.dtype, jnp.floating) else t)(jnp.asarray(a)))
    def _A_setup():
        B, Sq, D = 1, 1, 576
        Hq, Hkv, Sk, Dh = 32, 16, 65536, 128
        assert Hq % Hkv == 0, (Hq, Hkv)
        return {
            "x": _w((lambda *s: _rng.normal(s) * 0.05)(B, Sq, D)),
            "k_cache": _w((lambda *s: _rng.normal(s) * 0.05)(B, Hkv, Sk, Dh)),
            "v_cache": _w((lambda *s: _rng.normal(s) * 0.05)(B, Hkv, Sk, Dh)),
            "wq": _w((lambda *s: _rng.normal(s) * 0.05)(D, Hq * Dh) * (D ** -0.5)),
            "wo": _w((lambda *s: _rng.normal(s) * 0.05)(Hq * Dh, D) * ((Hq * Dh) ** -0.5)),
        }
    _A_in = _A_setup()

    def _B_setup():
        B, S, D, F = 1, 1, 576, 4608
        return {
            "x": _w((lambda *s: _rng.normal(s) * 0.05)(B, S, D)),
            "w_gate": _w((lambda *s: _rng.normal(s) * 0.05)(D, F)),
            "w_up": _w((lambda *s: _rng.normal(s) * 0.05)(D, F)),
            "w_down": _w((lambda *s: _rng.normal(s) * 0.05)(F, D)),
        }
    _B_in = _B_setup()

    return {
        "A_x": _A_in["x"],
        "A_k_cache": _A_in["k_cache"],
        "A_v_cache": _A_in["v_cache"],
        "A_wq": _A_in["wq"],
        "A_wo": _A_in["wo"],
        "B_x": _B_in["x"],
        "B_w_gate": _B_in["w_gate"],
        "B_w_up": _B_in["w_up"],
        "B_w_down": _B_in["w_down"],
    }

def reference(A_x, A_k_cache, A_v_cache, A_wq, A_wo, B_x, B_w_gate, B_w_up, B_w_down):
    def _A_ref(x, k_cache, v_cache, wq, wo):
        B, Sq, D = x.shape
        Hq, Dh = 32, 128
        Hkv, Sk = k_cache.shape[1], k_cache.shape[2]
        W = min(4096, max(256, Sk // 4))
        rep = Hq // Hkv
        q = (lambda x, *d: x.transpose(*d))((x @ wq).reshape(B, Sq, Hq, Dh), 0, 2, 1, 3)
        k = jnp.repeat(k_cache[:, :, Sk - W:, :], rep, axis=1)
        v = jnp.repeat(v_cache[:, :, Sk - W:, :], rep, axis=1)
        scores = jnp.einsum("bhqd,bhkd->bhqk", q, k) * (Dh ** -0.5)
        p = _softmax(scores, axis=-1)
        o = jnp.einsum("bhqk,bhkd->bhqd", p, v)
        return (lambda x, *d: x.transpose(*d))(o, 0, 2, 1, 3).reshape(B, Sq, Hq * Dh) @ wo

    def _B_ref(x, w_gate, w_up, w_down):
        g = jnp.einsum("bsd,df->bsf", x, w_gate)
        u = jnp.einsum("bsd,df->bsf", x, w_up)
        h = _sigmoid(g) * u
        return jnp.einsum("bsf,fd->bsd", h, w_down)

    x = A_x
    xn = _layernorm(x, axis=-1)
    s = _A_ref(xn, A_k_cache, A_v_cache, A_wq, A_wo)
    g = _silu(_B_ref(xn, B_w_gate, B_w_up, B_w_down))
    return x + s * g
```

```python
import jax
import jax.numpy as jnp
from jax import lax
import jax.experimental.pallas as pl
import jax.experimental.pallas.tpu as pltpu

_HQ = 32
_DH = 128
_NSLOT = 4
_NT = (((1,), (1,)), ((), ()))


def _make_kernel(D, Hkv, Sk, W, F, f_chunks):
    rep = _HQ // Hkv
    bf16, f32 = jnp.bfloat16, jnp.float32
    hw = rep * _DH
    assert rep <= 8 and sum(f_chunks) == F

    def kernel(x_hbm, k_hbm, v_hbm, wq_hbm, wo_hbm, wg_hbm, wu_hbm, wd_hbm,
               o_ref,
               xb, kb, vb, wqb, wob, wgb, wub, wdb, qs, os_, sems):
        def kv_group(h):
            sem = sems.at[(h + 1) % _NSLOT]
            return [
                pltpu.make_async_copy(k_hbm.at[0, h, pl.ds(Sk - W, W), :], kb.at[h], sem),
                pltpu.make_async_copy(v_hbm.at[0, h, pl.ds(Sk - W, W), :], vb.at[h], sem),
            ]

        def first_group():
            sem = sems.at[0]
            return [
                pltpu.make_async_copy(x_hbm, xb, sem),
                pltpu.make_async_copy(wq_hbm, wqb, sem),
            ]

        tail = []
        g = Hkv + 1
        tail.append([pltpu.make_async_copy(wo_hbm, wob, sems.at[g % _NSLOT])])
        c0 = 0
        for c in f_chunks:
            g += 1
            sem = sems.at[g % _NSLOT]
            cs = pl.ds(c0, c)
            tail.append([
                pltpu.make_async_copy(wg_hbm.at[:, cs], wgb.at[:, cs], sem),
                pltpu.make_async_copy(wu_hbm.at[:, cs], wub.at[:, cs], sem),
                pltpu.make_async_copy(wd_hbm.at[:, cs], wdb.at[:, cs], sem),
            ])
            c0 += c

        def start(group):
            for cp in group:
                cp.start()

        def wait(group):
            for cp in group:
                cp.wait()

        start(first_group())
        for h in range(_NSLOT - 1):
            start(kv_group(h))

        wait(first_group())
        start(kv_group(_NSLOT - 1))

        x = xb[0].astype(f32)
        mean = jnp.mean(x, axis=-1, keepdims=True)
        xc = x - mean
        var = jnp.mean(xc * xc, axis=-1, keepdims=True)
        xn = xc / jnp.sqrt(var + 1e-5)
        xn = jnp.broadcast_to(xn, (8, D)).astype(bf16)

        row = lax.broadcasted_iota(jnp.int32, (8, _DH), 0)
        q = jnp.dot(xn, wqb[...], preferred_element_type=f32)
        for h in range(Hkv):
            qh = q[:, h * hw:h * hw + _DH]
            for r in range(1, rep):
                qh = jnp.where(row == r, q[:, h * hw + r * _DH:h * hw + (r + 1) * _DH], qh)
            qs[h] = qh

        def attend(h):
            qh = qs[h].astype(bf16)
            s = lax.dot_general(qh, kb[h], _NT, preferred_element_type=f32)
            s = s * (_DH ** -0.5)
            m = jnp.max(s, axis=-1, keepdims=True)
            e = jnp.exp(s - m)
            l = jnp.sum(e, axis=-1, keepdims=True)
            o = jnp.dot(e.astype(bf16), vb[h], preferred_element_type=f32) / l
            for r in range(rep):
                os_[h * rep + r] = jnp.where(row == r, o, 0.0)

        def head(h, carry):
            wait(kv_group(h))
            start(kv_group(h + _NSLOT))
            attend(h)
            return carry

        lax.fori_loop(0, Hkv - _NSLOT, head, 0)
        for i in range(_NSLOT):
            h = Hkv - _NSLOT + i
            wait(kv_group(h))
            if i < len(tail):
                start(tail[i])
            attend(h)

        wait(tail[0])
        if _NSLOT < len(tail):
            start(tail[_NSLOT])
        o_all = jnp.concatenate([os_[j] for j in range(_HQ)], axis=-1).astype(bf16)
        s_acc = lax.dot_general(o_all, wob[...], _NT, preferred_element_type=f32)
        s_out = jnp.sum(s_acc, axis=0, keepdims=True)

        d_acc = jnp.zeros((8, D), f32)
        c0 = 0
        for j, c in enumerate(f_chunks):
            wait(tail[j + 1])
            if j + 1 + _NSLOT < len(tail):
                start(tail[j + 1 + _NSLOT])
            gate = jnp.dot(xn, wgb[:, c0:c0 + c], preferred_element_type=f32)
            up = jnp.dot(xn, wub[:, c0:c0 + c], preferred_element_type=f32)
            hid = (jax.nn.sigmoid(gate) * up).astype(bf16)
            d_acc = d_acc + lax.dot_general(
                hid, wdb[:, c0:c0 + c], _NT, preferred_element_type=f32)
            c0 += c

        d = d_acc[0:1]
        o_ref[0] = (x + s_out * (d * jax.nn.sigmoid(d))).astype(o_ref.dtype)

    return kernel


@jax.jit
def pallas_recurrent_scan__sliding_block_cached__glu_gated_glu__decode_kernel(
    A_x: jax.Array,
    A_k_cache: jax.Array,
    A_v_cache: jax.Array,
    A_wq: jax.Array,
    A_wo: jax.Array,
    B_x: jax.Array,
    B_w_gate: jax.Array,
    B_w_up: jax.Array,
    B_w_down: jax.Array,
):
    del B_x
    B, Sq, D = A_x.shape
    assert B == 1 and Sq == 1
    Hkv, Sk = A_k_cache.shape[1], A_k_cache.shape[2]
    W = min(4096, max(256, Sk // 4))
    F = B_w_gate.shape[1]
    f_chunks = (1024, 1024, 1024, 768, 512, 256)
    bf16 = jnp.bfloat16

    hbm = pl.BlockSpec(memory_space=pl.ANY)
    return pl.pallas_call(
        _make_kernel(D, Hkv, Sk, W, F, f_chunks),
        out_shape=jax.ShapeDtypeStruct(A_x.shape, A_x.dtype),
        in_specs=[hbm] * 8,
        out_specs=pl.BlockSpec(memory_space=pltpu.VMEM),
        scratch_shapes=[
            pltpu.VMEM(A_x.shape, A_x.dtype),
            pltpu.VMEM((Hkv, W, _DH), A_k_cache.dtype),
            pltpu.VMEM((Hkv, W, _DH), A_v_cache.dtype),
            pltpu.VMEM((D, _HQ * _DH), bf16),
            pltpu.VMEM((D, _HQ * _DH), bf16),
            pltpu.VMEM((D, F), bf16),
            pltpu.VMEM((D, F), bf16),
            pltpu.VMEM((D, F), bf16),
            pltpu.VMEM((Hkv, 8, _DH), jnp.float32),
            pltpu.VMEM((_HQ, 8, _DH), jnp.float32),
            pltpu.SemaphoreType.DMA((_NSLOT,)),
        ],
        compiler_params=pltpu.CompilerParams(vmem_limit_bytes=100 * 1024 * 1024),
    )(A_x, A_k_cache, A_v_cache, A_wq, A_wo.T, B_w_gate, B_w_up, B_w_down.T)
```

```python
import jax
import jax.numpy as jnp
from jax import lax
import jax.experimental.pallas as pl
import jax.experimental.pallas.tpu as pltpu

_HQ = 32
_DH = 128
_AHEAD = 8
_CW = 512
_RW = 32
_CK = 128
_RK = 64
_HK = 2
_NT = (((1,), (1,)), ((), ()))


def _make_kernel(D, Hkv, Sk, W, F):
    rep = _HQ // Hkv
    bf16, f32 = jnp.bfloat16, jnp.float32
    hw = rep * _DH
    hpb = _CW // hw
    nq, nf, nk = _HQ * _DH // _CW, F // _CW, W // _CK
    assert rep <= 8 and _CW % hw == 0 and F % _CW == 0 and W % _CK == 0
    assert D % _RW == 0 and Hkv % _HK == 0 and min(nq, nf, nk) >= _AHEAD

    def kernel(x_hbm, k_hbm, v_hbm, wq_hbm, wo_hbm, wg_hbm, wu_hbm, wd_hbm,
               o_ref,
               xb, kb, vb, wqb, wob, wgb, wub, wdb,
               qs, gs, hs, sc, ms, ls, acc, ob, sems, xsem):

        def aligned(i, n):
            return i * n if isinstance(i, int) else pl.multiple_of(i * n, n)

        def weight_stream(src, dst):
            def batch(i, sem):
                cols = pl.ds(aligned(i, _CW), _CW)
                return [
                    pltpu.make_async_copy(
                        src.at[pl.ds(r, _RW), cols], dst.at[pl.ds(r, _RW), cols], sem)
                    for r in range(0, D, _RW)
                ]

            def whole(i, sem):
                blk = dst.at[:, pl.ds(aligned(i, _CW), _CW)]
                return pltpu.make_async_copy(blk, blk, sem)

            return batch, whole, dst.shape[1] // _CW

        def cache_stream(src, dst):
            def batch(i, sem):
                j0 = aligned(i, _CK)
                return [
                    pltpu.make_async_copy(
                        src.at[0, pl.ds(h, _HK), pl.ds(Sk - W + r + j0, _RK), :],
                        dst.at[pl.ds(h, _HK), pl.ds(r + j0, _RK), :], sem)
                    for r in range(0, _CK, _RK) for h in range(0, Hkv, _HK)
                ]

            def whole(i, sem):
                blk = dst.at[:, pl.ds(aligned(i, _CK), _CK), :]
                return pltpu.make_async_copy(blk, blk, sem)

            return batch, whole, nk

        streams = [
            weight_stream(wq_hbm, wqb),
            weight_stream(wg_hbm, wgb),
            weight_stream(wu_hbm, wub),
            cache_stream(k_hbm, kb),
            cache_stream(v_hbm, vb),
            weight_stream(wd_hbm, wdb),
            weight_stream(wo_hbm, wob),
        ]
        first = [sum(s[2] for s in streams[:n]) for n in range(len(streams))]

        def enqueue(s, i):
            sem = sems.at[(first[s] + i) % _AHEAD]
            for n, cp in enumerate(streams[s][0](i, sem)):
                cp.start(priority=n % 2)

        def run_stream(s, consume):
            n = streams[s][2]

            def step(i, carry):
                streams[s][1](i, sems.at[(first[s] + i) % _AHEAD]).wait()
                if n > _AHEAD:
                    pl.when(i + _AHEAD < n)(lambda: enqueue(s, i + _AHEAD))
                if s + 1 < len(streams):
                    pl.when(i + _AHEAD >= n)(lambda: enqueue(s + 1, i + _AHEAD - n))
                consume(i, carry)
                return carry

            lax.fori_loop(0, n, step, 0)

        x_copy = pltpu.make_async_copy(x_hbm, xb, xsem)
        x_copy.start()
        lax.fori_loop(0, _AHEAD, lambda i, c: (enqueue(0, i), c)[1], 0)
        x_copy.wait()

        x = xb[0].astype(f32)
        xc = x - jnp.mean(x, axis=-1, keepdims=True)
        var = jnp.mean(xc * xc, axis=-1, keepdims=True)
        xn = jnp.broadcast_to(xc / jnp.sqrt(var + 1e-5), (8, D)).astype(bf16)
        row = lax.broadcasted_iota(jnp.int32, (8, _DH), 0)

        def cols(i):
            return pl.ds(aligned(i, _CW), _CW)

        def keys(i):
            return pl.ds(aligned(i, _CK), _CK)

        def q_block(i, _):
            q = jnp.dot(xn, wqb[:, cols(i)], preferred_element_type=f32)
            for h in range(hpb):
                qh = q[:, h * hw:h * hw + _DH]
                for r in range(1, rep):
                    c = h * hw + r * _DH
                    qh = jnp.where(row == r, q[:, c:c + _DH], qh)
                qs[i * hpb + h] = qh.astype(bf16)

        def gate_block(i, _):
            g = jnp.dot(xn, wgb[:, cols(i)], preferred_element_type=f32)
            gs[:, cols(i)] = jax.nn.sigmoid(g)

        def up_block(i, _):
            u = jnp.dot(xn, wub[:, cols(i)], preferred_element_type=f32)
            hs[:, cols(i)] = (gs[:, cols(i)] * u).astype(bf16)

        def score_block(i, _):
            for h in range(Hkv):
                s = lax.dot_general(qs[h], kb[h, keys(i), :], _NT,
                                    preferred_element_type=f32) * (_DH ** -0.5)
                sc[h, :, keys(i)] = s
                ms[h] = jnp.maximum(ms[h], s)

        def value_block(i, _):
            for h in range(Hkv):
                e = jnp.exp(sc[h, :, keys(i)] - ms[h])
                ls[h] += e
                acc[h] += jnp.dot(e.astype(bf16), vb[h, keys(i), :],
                                  preferred_element_type=f32)

        def down_block(i, _):
            ob[0] += lax.dot_general(hs[:, cols(i)], wdb[:, cols(i)], _NT,
                                     preferred_element_type=f32)

        def out_block(i, _):
            parts = []
            for h in range(hpb):
                hh = i * hpb + h
                o = acc[hh] / jnp.sum(ls[hh], axis=-1, keepdims=True)
                parts += [jnp.where(row == r, o, 0.0) for r in range(rep)]
            o = jnp.concatenate(parts, axis=-1).astype(bf16)
            ob[1] += lax.dot_general(o, wob[:, cols(i)], _NT,
                                     preferred_element_type=f32)

        ms[...] = jnp.full(ms.shape, -jnp.inf, f32)
        ls[...] = jnp.zeros(ls.shape, f32)
        acc[...] = jnp.zeros(acc.shape, f32)
        ob[...] = jnp.zeros(ob.shape, f32)

        run_stream(0, q_block)
        run_stream(1, gate_block)
        run_stream(2, up_block)
        run_stream(3, score_block)
        for h in range(Hkv):
            ms[h] = jnp.broadcast_to(jnp.max(ms[h], axis=-1, keepdims=True), (8, _CK))
        run_stream(4, value_block)
        run_stream(5, down_block)
        run_stream(6, out_block)

        d = ob[0, 0:1, :]
        s = jnp.sum(ob[1], axis=0, keepdims=True)
        o_ref[0] = (x + s * (d * jax.nn.sigmoid(d))).astype(o_ref.dtype)

    return kernel


@jax.jit
def pallas_recurrent_scan__sliding_block_cached__glu_gated_glu__decode_kernel(
    A_x: jax.Array,
    A_k_cache: jax.Array,
    A_v_cache: jax.Array,
    A_wq: jax.Array,
    A_wo: jax.Array,
    B_x: jax.Array,
    B_w_gate: jax.Array,
    B_w_up: jax.Array,
    B_w_down: jax.Array,
):
    del B_x
    B, Sq, D = A_x.shape
    assert B == 1 and Sq == 1
    Hkv, Sk = A_k_cache.shape[1], A_k_cache.shape[2]
    W = min(4096, max(256, Sk // 4))
    F = B_w_gate.shape[1]
    bf16, f32 = jnp.bfloat16, jnp.float32

    return pl.pallas_call(
        _make_kernel(D, Hkv, Sk, W, F),
        out_shape=jax.ShapeDtypeStruct(A_x.shape, A_x.dtype),
        in_specs=[pl.BlockSpec(memory_space=pl.ANY)] * 8,
        out_specs=pl.BlockSpec(memory_space=pltpu.VMEM),
        scratch_shapes=[
            pltpu.VMEM(A_x.shape, A_x.dtype),
            pltpu.VMEM((Hkv, W, _DH), A_k_cache.dtype),
            pltpu.VMEM((Hkv, W, _DH), A_v_cache.dtype),
            pltpu.VMEM((D, _HQ * _DH), bf16),
            pltpu.VMEM((D, _HQ * _DH), bf16),
            pltpu.VMEM((D, F), bf16),
            pltpu.VMEM((D, F), bf16),
            pltpu.VMEM((D, F), bf16),
            pltpu.VMEM((Hkv, 8, _DH), bf16),
            pltpu.VMEM((8, F), f32),
            pltpu.VMEM((8, F), bf16),
            pltpu.VMEM((Hkv, 8, W), f32),
            pltpu.VMEM((Hkv, 8, _CK), f32),
            pltpu.VMEM((Hkv, 8, _CK), f32),
            pltpu.VMEM((Hkv, 8, _DH), f32),
            pltpu.VMEM((2, 8, D), f32),
            pltpu.SemaphoreType.DMA((_AHEAD,)),
            pltpu.SemaphoreType.DMA(()),
        ],
        compiler_params=pltpu.CompilerParams(
            vmem_limit_bytes=100 * 1024 * 1024, disable_bounds_checks=True),
    )(A_x, A_k_cache, A_v_cache, A_wq, A_wo.T, B_w_gate, B_w_up, B_w_down.T)
```

```python
import jax
import jax.numpy as jnp
from jax import lax
import jax.experimental.pallas as pl
import jax.experimental.pallas.tpu as pltpu

_HQ = 32
_DH = 128
_AHEAD = 8
_CW = 512
_RW = 32
_RB = 8
_CK = 128
_RK = 64
_HK = 2
_NT = (((1,), (1,)), ((), ()))


def _make_kernel(D, Hkv, Sk, W, F):
    rep = _HQ // Hkv
    bf16, f32 = jnp.bfloat16, jnp.float32
    hw = rep * _DH
    hpb = _CW // hw
    nq, nf, nk = _HQ * _DH // _CW, F // _CW, W // _CK
    assert rep <= 8 and _CW % hw == 0 and F % _CW == 0 and W % _CK == 0
    assert D % _RW == 0 and D % (9 * _RB) == 0 and Hkv % _HK == 0

    def kernel(x_hbm, k_hbm, v_hbm, wq_hbm, wo_hbm, wg_hbm, wu_hbm, wd_hbm,
               o_ref,
               xb, kb, vb, wqb, wob, wgb, wub, wdb,
               qs, gs, hs, sc, ms, ls, acc, os_, ob, sems, xsem):

        def aligned(i, n, align):
            return i * n if isinstance(i, int) else pl.multiple_of(i * n, align)

        def band_stream(lanes, n):
            def batch(i):
                out = []
                for b in range(3):
                    for c in range(2):
                        for src, dst, r0 in lanes:
                            rows = pl.ds(r0 + b * _RB + aligned(i, 3 * _RB, _RB), _RB)
                            half = pl.ds(c * (src.shape[1] // 2), src.shape[1] // 2)
                            out.append((src.at[rows, half], dst.at[rows, half]))
                return out

            def landed(i):
                return [dst.at[pl.ds(r0 + aligned(i, 3 * _RB, _RB), 3 * _RB), :]
                        for _, dst, r0 in lanes]

            return batch, landed, n

        def column_stream(src, dst):
            def batch(i):
                return [(src.at[pl.ds(r, _RW), cols(i)], dst.at[pl.ds(r, _RW), cols(i)])
                        for r in range(0, D, _RW)]

            return batch, lambda i: [dst.at[:, cols(i)]], dst.shape[1] // _CW

        def cache_stream(src, dst):
            def batch(i):
                j0 = aligned(i, _CK, _CK)
                return [
                    (src.at[0, pl.ds(h, _HK), pl.ds(Sk - W + r + j0, _RK), :],
                     dst.at[pl.ds(h, _HK), pl.ds(r + j0, _RK), :])
                    for r in range(0, _CK, _RK) for h in range(0, Hkv, _HK)
                ]

            return batch, lambda i: [dst.at[:, keys(i), :]], nk

        def cols(i):
            return pl.ds(aligned(i, _CW, _CW), _CW)

        def keys(i):
            return pl.ds(aligned(i, _CK, _CK), _CK)

        streams = [
            band_stream([(wq_hbm, wqb, r0) for r0 in range(0, D, D // 3)], D // (9 * _RB)),
            band_stream([(wg_hbm, wgb, 0), (wu_hbm, wub, 0), (wd_hbm, wdb, 0)],
                        D // (3 * _RB)),
            cache_stream(k_hbm, kb),
            cache_stream(v_hbm, vb),
            column_stream(wo_hbm, wob),
        ]
        assert all(s[2] >= _AHEAD for s in streams)
        assert nq <= streams[1][2] and 3 * nf <= nk
        first = [sum(s[2] for s in streams[:n]) for n in range(len(streams))]

        def enqueue(s, i):
            sem = sems.at[(first[s] + i) % _AHEAD]
            for n, (src, dst) in enumerate(streams[s][0](i)):
                pltpu.make_async_copy(src, dst, sem).start(priority=n % 2)

        def run_stream(s, consume):
            n = streams[s][2]

            def step(i, carry):
                sem = sems.at[(first[s] + i) % _AHEAD]
                for region in streams[s][1](i):
                    pltpu.make_async_copy(region, region, sem).wait()
                if n > _AHEAD:
                    pl.when(i + _AHEAD < n)(lambda: enqueue(s, i + _AHEAD))
                if s + 1 < len(streams):
                    pl.when(i + _AHEAD >= n)(lambda: enqueue(s + 1, i + _AHEAD - n))
                consume(i)
                return carry

            lax.fori_loop(0, n, step, 0)

        x_copy = pltpu.make_async_copy(x_hbm, xb, xsem)
        x_copy.start()
        lax.fori_loop(0, _AHEAD, lambda i, c: (enqueue(0, i), c)[1], 0)

        ms[...] = jnp.full(ms.shape, -jnp.inf, f32)
        ls[...] = jnp.zeros(ls.shape, f32)
        acc[...] = jnp.zeros(acc.shape, f32)
        ob[...] = jnp.zeros(ob.shape, f32)

        x_copy.wait()
        x = xb[0].astype(f32)
        xc = x - jnp.mean(x, axis=-1, keepdims=True)
        var = jnp.mean(xc * xc, axis=-1, keepdims=True)
        xn = jnp.broadcast_to(xc / jnp.sqrt(var + 1e-5), (8, D)).astype(bf16)
        row = lax.broadcasted_iota(jnp.int32, (8, _DH), 0)

        def q_block(i):
            q = jnp.dot(xn, wqb[:, cols(i)], preferred_element_type=f32)
            for h in range(hpb):
                qh = q[:, h * hw:h * hw + _DH]
                for r in range(1, rep):
                    c = h * hw + r * _DH
                    qh = jnp.where(row == r, q[:, c:c + _DH], qh)
                qs[i * hpb + h] = qh.astype(bf16)

        def gate_block(i):
            g = jnp.dot(xn, wgb[:, cols(i)], preferred_element_type=f32)
            gs[:, cols(i)] = jax.nn.sigmoid(g)

        def up_block(i):
            u = jnp.dot(xn, wub[:, cols(i)], preferred_element_type=f32)
            hs[:, cols(i)] = (gs[:, cols(i)] * u).astype(bf16)

        def down_block(i):
            ob[0] += lax.dot_general(hs[:, cols(i)], wdb[:, cols(i)], _NT,
                                     preferred_element_type=f32)

        def score_block(i):
            for h in range(Hkv):
                s = lax.dot_general(qs[h], kb[h, keys(i), :], _NT,
                                    preferred_element_type=f32) * (_DH ** -0.5)
                sc[h, :, keys(i)] = s
                ms[h] = jnp.maximum(ms[h], s)
            for n, block in enumerate((gate_block, up_block, down_block)):
                pl.when((i >= n * nf) & (i < (n + 1) * nf))(
                    lambda n=n, block=block: block(i - n * nf))

        def value_block(i):
            for h in range(Hkv):
                e = jnp.exp(sc[h, :, keys(i)] - ms[h])
                ls[h] += e
                acc[h] += jnp.dot(e.astype(bf16), vb[h, keys(i), :],
                                  preferred_element_type=f32)

        def out_block(i):
            ob[1] += lax.dot_general(os_[:, cols(i)], wob[:, cols(i)], _NT,
                                     preferred_element_type=f32)

        run_stream(0, lambda i: None)
        run_stream(1, lambda i: pl.when(i < nq)(lambda: q_block(i)))
        run_stream(2, score_block)
        for h in range(Hkv):
            ms[h] = jnp.broadcast_to(jnp.max(ms[h], axis=-1, keepdims=True), (8, _CK))
        run_stream(3, value_block)
        for h in range(Hkv):
            o = acc[h] / jnp.sum(ls[h], axis=-1, keepdims=True)
            for r in range(rep):
                c = h * hw + r * _DH
                os_[:, c:c + _DH] = jnp.where(row == r, o, 0.0).astype(bf16)
        d = ob[0, 0:1, :]
        gate = d * jax.nn.sigmoid(d)
        run_stream(4, out_block)

        s = jnp.sum(ob[1], axis=0, keepdims=True)
        o_ref[0] = (x + s * gate).astype(o_ref.dtype)

    return kernel


@jax.jit
def pallas_recurrent_scan__sliding_block_cached__glu_gated_glu__decode_kernel(
    A_x: jax.Array,
    A_k_cache: jax.Array,
    A_v_cache: jax.Array,
    A_wq: jax.Array,
    A_wo: jax.Array,
    B_x: jax.Array,
    B_w_gate: jax.Array,
    B_w_up: jax.Array,
    B_w_down: jax.Array,
):
    del B_x
    B, Sq, D = A_x.shape
    assert B == 1 and Sq == 1
    Hkv, Sk = A_k_cache.shape[1], A_k_cache.shape[2]
    W = min(4096, max(256, Sk // 4))
    F = B_w_gate.shape[1]
    bf16, f32 = jnp.bfloat16, jnp.float32

    return pl.pallas_call(
        _make_kernel(D, Hkv, Sk, W, F),
        out_shape=jax.ShapeDtypeStruct(A_x.shape, A_x.dtype),
        in_specs=[pl.BlockSpec(memory_space=pl.ANY)] * 8,
        out_specs=pl.BlockSpec(memory_space=pltpu.VMEM),
        scratch_shapes=[
            pltpu.VMEM(A_x.shape, A_x.dtype),
            pltpu.VMEM((Hkv, W, _DH), A_k_cache.dtype),
            pltpu.VMEM((Hkv, W, _DH), A_v_cache.dtype),
            pltpu.VMEM((D, _HQ * _DH), bf16),
            pltpu.VMEM((D, _HQ * _DH), bf16),
            pltpu.VMEM((D, F), bf16),
            pltpu.VMEM((D, F), bf16),
            pltpu.VMEM((D, F), bf16),
            pltpu.VMEM((Hkv, 8, _DH), bf16),
            pltpu.VMEM((8, F), f32),
            pltpu.VMEM((8, F), bf16),
            pltpu.VMEM((Hkv, 8, W), f32),
            pltpu.VMEM((Hkv, 8, _CK), f32),
            pltpu.VMEM((Hkv, 8, _CK), f32),
            pltpu.VMEM((Hkv, 8, _DH), f32),
            pltpu.VMEM((8, _HQ * _DH), bf16),
            pltpu.VMEM((2, 8, D), f32),
            pltpu.SemaphoreType.DMA((_AHEAD,)),
            pltpu.SemaphoreType.DMA(()),
        ],
        compiler_params=pltpu.CompilerParams(
            vmem_limit_bytes=100 * 1024 * 1024, disable_bounds_checks=True),
    )(A_x, A_k_cache, A_v_cache, A_wq, A_wo.T, B_w_gate, B_w_up, B_w_down.T)
```

```python
import jax
import jax.numpy as jnp
from jax import lax
import jax.experimental.pallas as pl
import jax.experimental.pallas.tpu as pltpu

_HQ = 32
_DH = 128
_AHEAD = 8
_CW = 512
_RW = 32
_RB = 8
_CK = 128
_RK = 64
_HK = 2
_NT = (((1,), (1,)), ((), ()))


def _make_kernel(D, Hkv, Sk, W, F):
    rep = _HQ // Hkv
    bf16, f32 = jnp.bfloat16, jnp.float32
    hw = rep * _DH
    hpb = _CW // hw
    nq, nf, nk = _HQ * _DH // _CW, F // _CW, W // _CK
    assert rep <= 8 and _CW % hw == 0 and F % _CW == 0 and W % _CK == 0
    assert D % _RW == 0 and Hkv % _HK == 0

    def kernel(x_hbm, k_hbm, v_hbm, wq_hbm, wo_hbm, wg_hbm, wu_hbm, wd_hbm,
               o_ref,
               xb, kb, vb, wqb, wob, wgb, wub, wdb,
               qs, gs, hs, sc, ms, ls, acc, os_, ob, sems, xsem):

        def aligned(i, n, align):
            return i * n if isinstance(i, int) else pl.multiple_of(i * n, align)

        def band_stream(weights, parts, nb):
            lanes = [(src, dst, r0) for r0 in range(0, D, D // parts) for src, dst in weights]

            def batch(i):
                out = []
                for b in range(nb):
                    for c in range(2):
                        for src, dst, r0 in lanes:
                            rows = pl.ds(r0 + b * _RB + aligned(i, nb * _RB, _RB), _RB)
                            half = pl.ds(c * (src.shape[1] // 2), src.shape[1] // 2)
                            out.append((src.at[rows, half], dst.at[rows, half]))
                return out

            def landed(i):
                return [dst.at[pl.ds(r0 + aligned(i, nb * _RB, _RB), nb * _RB), :]
                        for _, dst, r0 in lanes]

            assert D % (parts * nb * _RB) == 0
            return batch, landed, D // (parts * nb * _RB)

        def column_stream(src, dst):
            def batch(i):
                return [(src.at[pl.ds(r, _RW), cols(i)], dst.at[pl.ds(r, _RW), cols(i)])
                        for r in range(0, D, _RW)]

            return batch, lambda i: [dst.at[:, cols(i)]], dst.shape[1] // _CW

        def cache_stream(src, dst):
            head_order = sorted(range(0, Hkv, _HK), key=lambda h: format(h, "016b")[::-1])

            def batch(i):
                j0 = aligned(i, _CK, _CK)
                return [
                    (src.at[0, pl.ds(h, _HK), pl.ds(Sk - W + r + j0, _RK), :],
                     dst.at[pl.ds(h, _HK), pl.ds(r + j0, _RK), :])
                    for r in range(0, _CK, _RK) for h in head_order
                ]

            return batch, lambda i: [dst.at[:, keys(i), :]], nk

        def cols(i):
            return pl.ds(aligned(i, _CW, _CW), _CW)

        def keys(i):
            return pl.ds(aligned(i, _CK, _CK), _CK)

        streams = [
            band_stream([(wq_hbm, wqb)], 3, 3),
            band_stream([(wg_hbm, wgb), (wu_hbm, wub), (wd_hbm, wdb)], 2, 2),
            cache_stream(k_hbm, kb),
            cache_stream(v_hbm, vb),
            column_stream(wo_hbm, wob),
        ]
        assert all(s[2] >= _AHEAD for s in streams)
        assert nq <= streams[1][2] and 3 * nf <= nk
        first = [sum(s[2] for s in streams[:n]) for n in range(len(streams))]

        def enqueue(s, i):
            sem = sems.at[(first[s] + i) % _AHEAD]
            for n, (src, dst) in enumerate(streams[s][0](i)):
                pltpu.make_async_copy(src, dst, sem).start(priority=n % 2)

        def run_stream(s, consume):
            n = streams[s][2]

            def step(i, carry):
                sem = sems.at[(first[s] + i) % _AHEAD]
                for region in streams[s][1](i):
                    pltpu.make_async_copy(region, region, sem).wait()
                if n > _AHEAD:
                    pl.when(i + _AHEAD < n)(lambda: enqueue(s, i + _AHEAD))
                if s + 1 < len(streams):
                    pl.when(i + _AHEAD >= n)(lambda: enqueue(s + 1, i + _AHEAD - n))
                consume(i)
                return carry

            lax.fori_loop(0, n, step, 0)

        x_copy = pltpu.make_async_copy(x_hbm, xb, xsem)
        x_copy.start()
        lax.fori_loop(0, _AHEAD, lambda i, c: (enqueue(0, i), c)[1], 0)

        ms[...] = jnp.full(ms.shape, -jnp.inf, f32)
        ls[...] = jnp.zeros(ls.shape, f32)
        acc[...] = jnp.zeros(acc.shape, f32)
        ob[...] = jnp.zeros(ob.shape, f32)

        x_copy.wait()
        x = xb[0].astype(f32)
        xc = x - jnp.mean(x, axis=-1, keepdims=True)
        var = jnp.mean(xc * xc, axis=-1, keepdims=True)
        xn = jnp.broadcast_to(xc / jnp.sqrt(var + 1e-5), (8, D)).astype(bf16)
        row = lax.broadcasted_iota(jnp.int32, (8, _DH), 0)

        def q_block(i):
            q = jnp.dot(xn, wqb[:, cols(i)], preferred_element_type=f32)
            for h in range(hpb):
                qh = q[:, h * hw:h * hw + _DH]
                for r in range(1, rep):
                    c = h * hw + r * _DH
                    qh = jnp.where(row == r, q[:, c:c + _DH], qh)
                qs[i * hpb + h] = qh.astype(bf16)

        def gate_block(i):
            g = jnp.dot(xn, wgb[:, cols(i)], preferred_element_type=f32)
            gs[:, cols(i)] = jax.nn.sigmoid(g)

        def up_block(i):
            u = jnp.dot(xn, wub[:, cols(i)], preferred_element_type=f32)
            hs[:, cols(i)] = (gs[:, cols(i)] * u).astype(bf16)

        def down_block(i):
            ob[0] += lax.dot_general(hs[:, cols(i)], wdb[:, cols(i)], _NT,
                                     preferred_element_type=f32)

        def score_block(i):
            for h in range(Hkv):
                s = lax.dot_general(qs[h], kb[h, keys(i), :], _NT,
                                    preferred_element_type=f32) * (_DH ** -0.5)
                sc[h, :, keys(i)] = s
                ms[h] = jnp.maximum(ms[h], s)
            for n, block in enumerate((gate_block, up_block, down_block)):
                pl.when((i >= n * nf) & (i < (n + 1) * nf))(
                    lambda n=n, block=block: block(i - n * nf))

        def value_block(i):
            for h in range(Hkv):
                e = jnp.exp(sc[h, :, keys(i)] - ms[h])
                ls[h] += e
                acc[h] += jnp.dot(e.astype(bf16), vb[h, keys(i), :],
                                  preferred_element_type=f32)

        def out_block(i):
            ob[1] += lax.dot_general(os_[:, cols(i)], wob[:, cols(i)], _NT,
                                     preferred_element_type=f32)

        run_stream(0, lambda i: None)
        run_stream(1, lambda i: pl.when(i < nq)(lambda: q_block(i)))
        run_stream(2, score_block)
        for h in range(Hkv):
            ms[h] = jnp.broadcast_to(jnp.max(ms[h], axis=-1, keepdims=True), (8, _CK))
        run_stream(3, value_block)
        for h in range(Hkv):
            o = acc[h] / jnp.sum(ls[h], axis=-1, keepdims=True)
            for r in range(rep):
                c = h * hw + r * _DH
                os_[:, c:c + _DH] = jnp.where(row == r, o, 0.0).astype(bf16)
        d = ob[0, 0:1, :]
        gate = d * jax.nn.sigmoid(d)
        run_stream(4, out_block)

        s = jnp.sum(ob[1], axis=0, keepdims=True)
        o_ref[0] = (x + s * gate).astype(o_ref.dtype)

    return kernel


@jax.jit
def pallas_recurrent_scan__sliding_block_cached__glu_gated_glu__decode_kernel(
    A_x: jax.Array,
    A_k_cache: jax.Array,
    A_v_cache: jax.Array,
    A_wq: jax.Array,
    A_wo: jax.Array,
    B_x: jax.Array,
    B_w_gate: jax.Array,
    B_w_up: jax.Array,
    B_w_down: jax.Array,
):
    del B_x
    B, Sq, D = A_x.shape
    assert B == 1 and Sq == 1
    Hkv, Sk = A_k_cache.shape[1], A_k_cache.shape[2]
    W = min(4096, max(256, Sk // 4))
    F = B_w_gate.shape[1]
    bf16, f32 = jnp.bfloat16, jnp.float32

    return pl.pallas_call(
        _make_kernel(D, Hkv, Sk, W, F),
        out_shape=jax.ShapeDtypeStruct(A_x.shape, A_x.dtype),
        in_specs=[pl.BlockSpec(memory_space=pl.ANY)] * 8,
        out_specs=pl.BlockSpec(memory_space=pltpu.VMEM),
        scratch_shapes=[
            pltpu.VMEM(A_x.shape, A_x.dtype),
            pltpu.VMEM((Hkv, W, _DH), A_k_cache.dtype),
            pltpu.VMEM((Hkv, W, _DH), A_v_cache.dtype),
            pltpu.VMEM((D, _HQ * _DH), bf16),
            pltpu.VMEM((D, _HQ * _DH), bf16),
            pltpu.VMEM((D, F), bf16),
            pltpu.VMEM((D, F), bf16),
            pltpu.VMEM((D, F), bf16),
            pltpu.VMEM((Hkv, 8, _DH), bf16),
            pltpu.VMEM((8, F), f32),
            pltpu.VMEM((8, F), bf16),
            pltpu.VMEM((Hkv, 8, W), f32),
            pltpu.VMEM((Hkv, 8, _CK), f32),
            pltpu.VMEM((Hkv, 8, _CK), f32),
            pltpu.VMEM((Hkv, 8, _DH), f32),
            pltpu.VMEM((8, _HQ * _DH), bf16),
            pltpu.VMEM((2, 8, D), f32),
            pltpu.SemaphoreType.DMA((_AHEAD,)),
            pltpu.SemaphoreType.DMA(()),
        ],
        compiler_params=pltpu.CompilerParams(
            vmem_limit_bytes=100 * 1024 * 1024),
    )(A_x, A_k_cache, A_v_cache, A_wq, A_wo.T, B_w_gate, B_w_up, B_w_down.T)
```

```python
import jax
import jax.numpy as jnp
from jax import lax
import jax.experimental.pallas as pl
import jax.experimental.pallas.tpu as pltpu

_HQ = 32
_DH = 128
_AHEAD = 8
_CW = 512
_RW = 32
_RB = 8
_CK = 128
_RK = 64
_HK = 2
_NT = (((1,), (1,)), ((), ()))


def _make_kernel(D, Hkv, Sk, W, F):
    rep = _HQ // Hkv
    bf16, f32 = jnp.bfloat16, jnp.float32
    hw = rep * _DH
    hpb = _CW // hw
    nq, nf, nk = _HQ * _DH // _CW, F // _CW, W // _CK
    assert rep <= 8 and _CW % hw == 0 and F % _CW == 0 and W % _CK == 0
    assert D % _RW == 0 and Hkv % _HK == 0

    def kernel(x_hbm, k_hbm, v_hbm, wq_hbm, wo_hbm, wg_hbm, wu_hbm, wd_hbm,
               o_ref,
               xb, kb, vb, wqb, wob, wgb, wub, wdb,
               qs, gs, hs, sc, ms, ls, acc, os_, ob, sems, xsem):

        def aligned(i, n, align):
            return i * n if isinstance(i, int) else pl.multiple_of(i * n, align)

        def band_stream(weights, parts, nb):
            lanes = [(src, dst, r0) for r0 in range(0, D, D // parts) for src, dst in weights]

            def batch(i):
                out = []
                for b in range(nb):
                    for c in range(2):
                        for src, dst, r0 in lanes:
                            rows = pl.ds(r0 + b * _RB + aligned(i, nb * _RB, _RB), _RB)
                            half = pl.ds(c * (src.shape[1] // 2), src.shape[1] // 2)
                            out.append((src.at[rows, half], dst.at[rows, half]))
                return out

            assert D % (parts * nb * _RB) == 0
            return batch, D // (parts * nb * _RB)

        def column_stream(src, dst):
            def batch(i):
                return [(src.at[pl.ds(r, _RW), cols(i)], dst.at[pl.ds(r, _RW), cols(i)])
                        for r in range(0, D, _RW)]

            return batch, dst.shape[1] // _CW

        def cache_stream(src, dst):
            head_order = sorted(range(0, Hkv, _HK), key=lambda h: format(h, "016b")[::-1])

            def batch(i):
                j0 = aligned(i, _CK, _CK)
                return [
                    (src.at[0, pl.ds(h, _HK), pl.ds(Sk - W + r + j0, _RK), :],
                     dst.at[pl.ds(h, _HK), pl.ds(r + j0, _RK), :])
                    for r in range(0, _CK, _RK) for h in head_order
                ]

            return batch, nk

        def cols(i):
            return pl.ds(aligned(i, _CW, _CW), _CW)

        def keys(i):
            return pl.ds(aligned(i, _CK, _CK), _CK)

        streams = [
            band_stream([(wq_hbm, wqb)], 3, 3),
            band_stream([(wg_hbm, wgb), (wu_hbm, wub), (wd_hbm, wdb)], 2, 2),
            cache_stream(k_hbm, kb),
            cache_stream(v_hbm, vb),
            column_stream(wo_hbm, wob),
        ]
        assert all(n >= _AHEAD for _, n in streams)
        assert nq <= streams[1][1] and 3 * nf <= nk
        first = [sum(n for _, n in streams[:s]) for s in range(len(streams))]

        def copies(s, i):
            sem = sems.at[(first[s] + i) % _AHEAD]
            return [pltpu.make_async_copy(src, dst, sem) for src, dst in streams[s][0](i)]

        def enqueue(s, i):
            for n, cp in enumerate(copies(s, i)):
                cp.start(priority=n % 2)

        def run_stream(s, consume):
            n = streams[s][1]

            def step(i, carry):
                for cp in copies(s, i):
                    cp.wait()
                if n > _AHEAD:
                    pl.when(i + _AHEAD < n)(lambda: enqueue(s, i + _AHEAD))
                if s + 1 < len(streams):
                    pl.when(i + _AHEAD >= n)(lambda: enqueue(s + 1, i + _AHEAD - n))
                consume(i)
                return carry

            lax.fori_loop(0, n, step, 0)

        x_copy = pltpu.make_async_copy(x_hbm, xb, xsem)
        x_copy.start()
        lax.fori_loop(0, _AHEAD, lambda i, c: (enqueue(0, i), c)[1], 0)

        ms[...] = jnp.full(ms.shape, -jnp.inf, f32)
        ls[...] = jnp.zeros(ls.shape, f32)
        acc[...] = jnp.zeros(acc.shape, f32)
        ob[...] = jnp.zeros(ob.shape, f32)

        x_copy.wait()
        x = xb[0].astype(f32)
        xc = x - jnp.mean(x, axis=-1, keepdims=True)
        var = jnp.mean(xc * xc, axis=-1, keepdims=True)
        xn = jnp.broadcast_to(xc / jnp.sqrt(var + 1e-5), (8, D)).astype(bf16)
        row = lax.broadcasted_iota(jnp.int32, (8, _DH), 0)

        def q_block(i):
            q = jnp.dot(xn, wqb[:, cols(i)], preferred_element_type=f32)
            for h in range(hpb):
                qh = q[:, h * hw:h * hw + _DH]
                for r in range(1, rep):
                    c = h * hw + r * _DH
                    qh = jnp.where(row == r, q[:, c:c + _DH], qh)
                qs[i * hpb + h] = qh.astype(bf16)

        def gate_block(i):
            g = jnp.dot(xn, wgb[:, cols(i)], preferred_element_type=f32)
            gs[:, cols(i)] = jax.nn.sigmoid(g)

        def up_block(i):
            u = jnp.dot(xn, wub[:, cols(i)], preferred_element_type=f32)
            hs[:, cols(i)] = (gs[:, cols(i)] * u).astype(bf16)

        def down_block(i):
            ob[0] += lax.dot_general(hs[:, cols(i)], wdb[:, cols(i)], _NT,
                                     preferred_element_type=f32)

        def score_block(i):
            for h in range(Hkv):
                s = lax.dot_general(qs[h], kb[h, keys(i), :], _NT,
                                    preferred_element_type=f32) * (_DH ** -0.5)
                sc[h, :, keys(i)] = s
                ms[h] = jnp.maximum(ms[h], s)
            for n, block in enumerate((gate_block, up_block, down_block)):
                pl.when((i >= n * nf) & (i < (n + 1) * nf))(
                    lambda n=n, block=block: block(i - n * nf))

        def value_block(i):
            for h in range(Hkv):
                e = jnp.exp(sc[h, :, keys(i)] - ms[h])
                ls[h] += e
                acc[h] += jnp.dot(e.astype(bf16), vb[h, keys(i), :],
                                  preferred_element_type=f32)

        def out_block(i):
            ob[1] += lax.dot_general(os_[:, cols(i)], wob[:, cols(i)], _NT,
                                     preferred_element_type=f32)

        run_stream(0, lambda i: None)
        run_stream(1, lambda i: pl.when(i < nq)(lambda: q_block(i)))
        run_stream(2, score_block)
        for h in range(Hkv):
            ms[h] = jnp.broadcast_to(jnp.max(ms[h], axis=-1, keepdims=True), (8, _CK))
        run_stream(3, value_block)
        for h in range(Hkv):
            o = acc[h] / jnp.sum(ls[h], axis=-1, keepdims=True)
            for r in range(rep):
                c = h * hw + r * _DH
                os_[:, c:c + _DH] = jnp.where(row == r, o, 0.0).astype(bf16)
        d = ob[0, 0:1, :]
        gate = d * jax.nn.sigmoid(d)
        run_stream(4, out_block)

        s = jnp.sum(ob[1], axis=0, keepdims=True)
        o_ref[0] = (x + s * gate).astype(o_ref.dtype)

    return kernel


@jax.jit
def pallas_recurrent_scan__sliding_block_cached__glu_gated_glu__decode_kernel(
    A_x: jax.Array,
    A_k_cache: jax.Array,
    A_v_cache: jax.Array,
    A_wq: jax.Array,
    A_wo: jax.Array,
    B_x: jax.Array,
    B_w_gate: jax.Array,
    B_w_up: jax.Array,
    B_w_down: jax.Array,
):
    del B_x
    B, Sq, D = A_x.shape
    assert B == 1 and Sq == 1
    Hkv, Sk = A_k_cache.shape[1], A_k_cache.shape[2]
    W = min(4096, max(256, Sk // 4))
    F = B_w_gate.shape[1]
    bf16, f32 = jnp.bfloat16, jnp.float32

    return pl.pallas_call(
        _make_kernel(D, Hkv, Sk, W, F),
        out_shape=jax.ShapeDtypeStruct(A_x.shape, A_x.dtype),
        in_specs=[pl.BlockSpec(memory_space=pl.ANY)] * 8,
        out_specs=pl.BlockSpec(memory_space=pltpu.VMEM),
        scratch_shapes=[
            pltpu.VMEM(A_x.shape, A_x.dtype),
            pltpu.VMEM((Hkv, W, _DH), A_k_cache.dtype),
            pltpu.VMEM((Hkv, W, _DH), A_v_cache.dtype),
            pltpu.VMEM((D, _HQ * _DH), bf16),
            pltpu.VMEM((D, _HQ * _DH), bf16),
            pltpu.VMEM((D, F), bf16),
            pltpu.VMEM((D, F), bf16),
            pltpu.VMEM((D, F), bf16),
            pltpu.VMEM((Hkv, 8, _DH), bf16),
            pltpu.VMEM((8, F), f32),
            pltpu.VMEM((8, F), bf16),
            pltpu.VMEM((Hkv, 8, W), f32),
            pltpu.VMEM((Hkv, 8, _CK), f32),
            pltpu.VMEM((Hkv, 8, _CK), f32),
            pltpu.VMEM((Hkv, 8, _DH), f32),
            pltpu.VMEM((8, _HQ * _DH), bf16),
            pltpu.VMEM((2, 8, D), f32),
            pltpu.SemaphoreType.DMA((_AHEAD,)),
            pltpu.SemaphoreType.DMA(()),
        ],
        compiler_params=pltpu.CompilerParams(
            vmem_limit_bytes=100 * 1024 * 1024),
    )(A_x, A_k_cache, A_v_cache, A_wq, A_wo.T, B_w_gate, B_w_up, B_w_down.T)
```
